```python
import os as _os
_os.environ.setdefault("JAX_PLATFORMS", "cpu")
import jax
import jax.numpy as jnp

def _softmax(x, axis=-1):
    return jax.nn.softmax(x, axis=axis)
def _gelu(x):
    return jax.nn.gelu(x, approximate=True)
def _silu(x):
    return jax.nn.silu(x)
def _sigmoid(x):
    return jax.nn.sigmoid(x)
def _layernorm(x, axis=-1, eps=1e-5):
    m = jnp.mean(x, axis=axis, keepdims=True)
    v = jnp.var(x, axis=axis, keepdims=True)
    return (x - m) / jnp.sqrt(v + eps)
def _scatter_add(tgt, idx, src, axis=0):
    return tgt.at[idx].add(src)
def _segment_sum(src, seg, n):
    return jax.ops.segment_sum(src, seg, n)
class _Rng:
    def __init__(self, key):
        self._k = key
    def _next(self):
        self._k, sub = jax.random.split(self._k)
        return sub
    def normal(self, shape):
        return jax.random.normal(self._next(), shape, dtype=jnp.bfloat16)
    def randint(self, lo, hi, shape):
        return jax.random.randint(self._next(), shape, lo, hi, dtype=jnp.int32)
    def uniform(self, shape, lo=0.0, hi=1.0):
        return jax.random.uniform(self._next(), shape, jnp.bfloat16, lo, hi)
    def permutation(self, n):
        return jax.random.permutation(self._next(), n)


kernel_name = 'gated_mix__compressed_kv_cla__linear_attn_block__prompt'

def setup_inputs():
    _rng = _Rng(jax.random.key(int.from_bytes(__import__("os").urandom(4), "little")))
    _w = (lambda a: (lambda t: t.astype(jnp.bfloat16) if jnp.issubdtype(t.dtype, jnp.floating) else t)(jnp.asarray(a)))
    def _A_setup():
        B, H, Sq, Sk, D, M = 1, 16, 2048, 2048, 256, 448
        Dc = 4 * D
        return {
            "x": _w((lambda *s: _rng.normal(s) * 0.05)(B, Sq, M)),
            "c_kv": _w((lambda *s: _rng.normal(s) * 0.8)(B, Sk, Dc)),
            "w_q": _w((lambda *s: _rng.normal(s) * 3.2)(M, H, D) * (M ** -0.5)),
            "w_uk": _w((lambda *s: _rng.normal(s) * 3.2)(Dc, H, D) * (Dc ** -0.5)),
            "w_uv": _w((lambda *s: _rng.normal(s) * 0.8)(Dc, H, D) * (Dc ** -0.5)),
            "w_o": _w((lambda *s: _rng.normal(s) * 0.8)(H, D, M) * ((H * D) ** -0.5)),
        }
    _A_in = _A_setup()

    def _B_setup():
        B, S, D = 1, 2048, 448
        return {
            "x": _w((lambda *s: _rng.normal(s) * 0.05)(B, S, D)),
            "wqkv": _w((lambda *s: _rng.normal(s) * 1.6)(D, 3 * D)),
            "wo": _w((lambda *s: _rng.normal(s) * 0.4)(D, D)),
        }
    _B_in = _B_setup()

    return {
        "A_x": _A_in["x"],
        "A_c_kv": _A_in["c_kv"],
        "A_w_q": _A_in["w_q"],
        "A_w_uk": _A_in["w_uk"],
        "A_w_uv": _A_in["w_uv"],
        "A_w_o": _A_in["w_o"],
        "B_x": _B_in["x"],
        "B_wqkv": _B_in["wqkv"],
        "B_wo": _B_in["wo"],
        "gate_w": _w((lambda *s: _rng.normal(s) * 0.05)(448) * 16.0),
    }

def reference(A_x, A_c_kv, A_w_q, A_w_uk, A_w_uv, A_w_o, B_x, B_wqkv, B_wo, gate_w):
    def _A_ref(x, c_kv, w_q, w_uk, w_uv, w_o):
        B, Sq, M = x.shape[0], x.shape[1], x.shape[2]
        Sk = c_kv.shape[1]
        H, D = w_q.shape[1], w_q.shape[2]
        q = jnp.einsum("bqm,mhd->bhqd", x, w_q)
        k = jnp.einsum("bkc,chd->bhkd", c_kv, w_uk)
        v = jnp.einsum("bkc,chd->bhkd", c_kv, w_uv)
        scores = jnp.einsum("bhqd,bhkd->bhqk", q, k) * (D ** -0.5)
        off = Sk - Sq
        qi = jnp.arange(Sq)[:, None]
        kj = jnp.arange(Sk)[None, :]
        cmask = kj <= (qi + off)
        scores = jnp.where(cmask[None, None], scores, -1e9)
        p = _softmax(scores, axis=-1)
        ctx = jnp.einsum("bhqk,bhkd->bhqd", p, v)
        return jnp.einsum("bhqd,hdm->bqm", ctx, w_o)

    def _B_ref(x, wqkv, wo):
        B, S, D = x.shape
        H = 16; Dh = D // H
        qkv = (lambda x, *d: x.transpose(*d))((x @ wqkv).reshape(B, S, 3, H, Dh), 2, 0, 3, 1, 4)
        q, k, v = qkv[0], qkv[1], qkv[2]
        phi = lambda t: jnp.where(t > 0, t + 1, jnp.exp(t)) + 1e-6
        pq, pk = phi(q), phi(k)
        kv = jnp.einsum("bhsd,bhse->bhde", pk, v)
        z = jnp.einsum("bhsd->bhd", pk)
        num = jnp.einsum("bhqd,bhde->bhqe", pq, kv)
        den = jnp.einsum("bhqd,bhd->bhq", pq, z)[..., None] + 1e-6
        o = num / den
        return (lambda x, *d: x.transpose(*d))(o, 0, 2, 1, 3).reshape(B, S, D) @ wo

    x = A_x
    g = _sigmoid((x * gate_w).sum(-1, keepdims=True))
    a = _A_ref(x, A_c_kv, A_w_q, A_w_uk, A_w_uv, A_w_o)
    b = _B_ref(x, B_wqkv, B_wo)
    return g * a + (1 - g) * b
```

```python
import jax
import jax.numpy as jnp
from jax import lax
import jax.experimental.pallas as pl
import jax.experimental.pallas.tpu as pltpu

S = 2048
M = 448
H = 16
D = 256
DC = 1024
DH = 28
TQ = 256
NQ = S // TQ
RC = 512
CB = 512
MG = 3 * M + 16
MV = M + 16

f32 = jnp.float32
bf16 = jnp.bfloat16
NT = (((1,), (1,)), ((), ()))


def _dot(a, b):
    return jnp.dot(a, b, preferred_element_type=f32)


def _dot_nt(a, b):
    return lax.dot_general(a, b, NT, preferred_element_type=f32)


def _phi(t):
    return jnp.where(t > 0, t + 1.0, jnp.exp(t)) + 1e-6


def kernel(xt_hbm, c_hbm, wq_hbm, wk_hbm, wv_hbm, wot_hbm, wqkv_hbm, wob_hbm, g_hbm, o_ref,
           xt_v, c_v, wq_v, wk_v, wv_v, wot_v, wqkv_v, wob_v, g_v, sems,
           x_s, wq_s, wk_s, wv_s, q_s, k_s, v_s, ctx_s, acc_s,
           wg_s, wobt_s, pq_s, kv_s, w2_s, gate_s, accb_s):
    h = pl.program_id(0)

    srcs = (xt_hbm, wqkv_hbm, wob_hbm, g_hbm, wq_hbm, c_hbm, wk_hbm, wv_hbm, wot_hbm)
    dsts = (xt_v, wqkv_v, wob_v, g_v, wq_v, c_v, wk_v, wv_v, wot_v)
    copies = [pltpu.make_async_copy(s, d, sems.at[i]) for i, (s, d) in enumerate(zip(srcs, dsts))]

    @pl.when(h == 0)
    def _():
        for cp in copies:
            cp.start()
        for cp in copies[:4]:
            cp.wait()
        wg_s[0:3 * M, :] = wqkv_v[...].T
        wg_s[3 * M:MG, :] = jnp.broadcast_to(g_v[...], (16, M))
        wobt_s[...] = wob_v[...].T
        kv_s[...] = jnp.zeros_like(kv_s)

        def b1(j, carry):
            cs = pl.ds(pl.multiple_of(j * CB, CB), CB)
            xt_c = xt_v[0, :, cs]
            t = _dot(wg_s[...], xt_c)
            pq_s[:, cs] = _phi(t[0:M]).astype(bf16)
            pk = _phi(t[M:2 * M]).astype(bf16)
            vt = jnp.concatenate([t[2 * M:3 * M].astype(bf16), jnp.ones((16, CB), bf16)], axis=0)
            kv_s[...] += _dot_nt(vt, pk)
            gate_s[:, cs] = jax.nn.sigmoid(t[3 * M:3 * M + 8])
            x_s[cs, :] = xt_c.T
            return carry
        lax.fori_loop(0, S // CB, b1, 0)

        r = lax.broadcasted_iota(jnp.int32, (M, M), 0) // DH
        cc = lax.broadcasted_iota(jnp.int32, (M, M), 1) // DH
        bm = r == cc
        w2_s[0:M, :] = jnp.where(bm, kv_s[0:M, :], 0.0).astype(bf16)
        w2_s[M:2 * M, :] = jnp.where(bm, kv_s[M:M + 1, :], 0.0).astype(bf16)

        def b2(j, carry):
            cs = pl.ds(pl.multiple_of(j * CB, CB), CB)
            nd = _dot(w2_s[...], pq_s[:, cs])
            ot = (nd[0:M] / (nd[M:2 * M] + 1e-6)).astype(bf16)
            bt = _dot(wobt_s[...], ot)
            accb_s[:, cs] = (1.0 - gate_s[0:1, cs]) * bt
            return carry
        lax.fori_loop(0, S // CB, b2, 0)

        acc_s[...] = jnp.zeros_like(acc_s)
        for cp in copies[4:]:
            cp.wait()

        def rl_q(j, carry):
            rs = pl.ds(pl.multiple_of(j * 64, 64), 64)
            wq_s[rs, :] = wq_v[rs].reshape(64, H * D)
            return carry
        lax.fori_loop(0, M // 64, rl_q, 0)

        def rl_kv(j, carry):
            rs = pl.ds(pl.multiple_of(j * 64, 64), 64)
            wk_s[rs, :] = wk_v[rs].reshape(64, H * D)
            wv_s[rs, :] = wv_v[rs].reshape(64, H * D)
            return carry
        lax.fori_loop(0, DC // 64, rl_kv, 0)

    col = pl.ds(pl.multiple_of(h * D, D), D)

    def proj(r, carry):
        rs = pl.ds(pl.multiple_of(r * RC, RC), RC)
        q_s[rs, :] = (_dot(x_s[rs, :], wq_s[:, col]) * (D ** -0.5)).astype(bf16)
        c = c_v[0, rs, :]
        k_s[rs, :] = _dot(c, wk_s[:, col]).astype(bf16)
        v_s[rs, :] = _dot(c, wv_s[:, col]).astype(bf16)
        return carry
    lax.fori_loop(0, S // RC, proj, 0)

    row = lax.broadcasted_iota(jnp.int32, (TQ, TQ), 0)
    colid = lax.broadcasted_iota(jnp.int32, (TQ, TQ), 1)
    cmask = colid <= row

    for i in range(NQ):
        q = q_s[i * TQ:(i + 1) * TQ, :]
        sd = _dot_nt(q, k_s[i * TQ:(i + 1) * TQ, :])
        sd = jnp.where(cmask, sd, -1e9)
        m = jnp.max(sd, axis=-1, keepdims=True)
        if i > 0:
            so = _dot_nt(q, k_s[0:i * TQ, :])
            m = jnp.maximum(m, jnp.max(so, axis=-1, keepdims=True))
        pd = jnp.exp(sd - m)
        l = jnp.sum(pd, axis=-1, keepdims=True)
        ctx = _dot(pd.astype(bf16), v_s[i * TQ:(i + 1) * TQ, :])
        if i > 0:
            po = jnp.exp(so - m)
            l = l + jnp.sum(po, axis=-1, keepdims=True)
            ctx = ctx + _dot(po.astype(bf16), v_s[0:i * TQ, :])
        ctx_s[i * TQ:(i + 1) * TQ, :] = (ctx / l).astype(bf16)

    acc_s[...] += _dot_nt(wot_v[h], ctx_s[...])

    @pl.when(h == H - 1)
    def _():
        o_ref[0] = (gate_s[0:1, :] * acc_s[...] + accb_s[...]).astype(o_ref.dtype)


@jax.jit
def pallas_gated_mix__compressed_kv_cla__linear_attn_block__prompt_kernel(A_x, A_c_kv, A_w_q, A_w_uk, A_w_uv, A_w_o, B_x, B_wqkv, B_wo, gate_w):
    args = (jnp.swapaxes(A_x, 1, 2), A_c_kv, A_w_q, A_w_uk, A_w_uv, jnp.swapaxes(A_w_o, 1, 2),
            B_wqkv, B_wo, gate_w.reshape(1, M))
    out_t = pl.pallas_call(
        kernel,
        grid=(H,),
        in_specs=[pl.BlockSpec(memory_space=pl.ANY) for _ in args],
        out_specs=pl.BlockSpec((1, M, S), lambda h: (0, 0, 0)),
        out_shape=jax.ShapeDtypeStruct((1, M, S), bf16),
        scratch_shapes=[pltpu.VMEM(a.shape, a.dtype) for a in args] + [
            pltpu.SemaphoreType.DMA((len(args),)),
            pltpu.VMEM((S, M), bf16),
            pltpu.VMEM((M, H * D), bf16),
            pltpu.VMEM((DC, H * D), bf16),
            pltpu.VMEM((DC, H * D), bf16),
            pltpu.VMEM((S, D), bf16),
            pltpu.VMEM((S, D), bf16),
            pltpu.VMEM((S, D), bf16),
            pltpu.VMEM((S, D), bf16),
            pltpu.VMEM((M, S), f32),
            pltpu.VMEM((MG, M), bf16),
            pltpu.VMEM((M, M), bf16),
            pltpu.VMEM((M, S), bf16),
            pltpu.VMEM((MV, M), f32),
            pltpu.VMEM((2 * M, M), bf16),
            pltpu.VMEM((8, S), f32),
            pltpu.VMEM((M, S), f32),
        ],
        compiler_params=pltpu.CompilerParams(
            dimension_semantics=("arbitrary",),
            vmem_limit_bytes=110 * 1024 * 1024,
        ),
    )(*args)
    return jnp.swapaxes(out_t, 1, 2)
```

```python
import jax
import jax.numpy as jnp
from jax import lax
import jax.experimental.pallas as pl
import jax.experimental.pallas.tpu as pltpu

S = 2048
M = 448
H = 16
D = 256
DC = 1024
DH = 28
T = 128
NTILE = S // T
CB = 512
NCB = S // CB
MG = 3 * M + 16
MV = M + 16
RL = 64

f32 = jnp.float32
bf16 = jnp.bfloat16
NT = (((1,), (1,)), ((), ()))
TN = (((0,), (0,)), ((), ()))


def _dot(a, b):
    return jnp.dot(a, b, preferred_element_type=f32)


def _dot_nt(a, b):
    return lax.dot_general(a, b, NT, preferred_element_type=f32)


def _phi(t):
    return jnp.where(t > 0, t + 1.0, jnp.exp(t)) + 1e-6


def kernel(xt_hbm, c_hbm, wq_hbm, wk_hbm, wv_hbm, wot_hbm, wqkv_hbm, wob_hbm, g_hbm, o_hbm,
           xt_v, c_v, wq_v, wk_v, wv_v, wot_v, wqkv_v, wob_v, g_v, sems, osems,
           x_s, wq_s, wk_s, wv_s, q_s, k_s, v_s, ctx_s, acc_s,
           wg_s, pq_s, kv_s, w3_s, zm_s, gate_s, accb_s, s_s, p_s, l_s, o_s):
    h = pl.program_id(0)

    srcs = (wqkv_hbm, g_hbm, wob_hbm, wk_hbm, wv_hbm, wq_hbm, c_hbm, wot_hbm, xt_hbm)
    dsts = (wqkv_v, g_v, wob_v, wk_v, wv_v, wq_v, c_v, wot_v, xt_v)
    copies = [pltpu.make_async_copy(s, d, sems.at[i]) for i, (s, d) in enumerate(zip(srcs, dsts))]

    def relayout(dst, src, nrows):
        def body(j, carry):
            rs = pl.ds(pl.multiple_of(j * RL, RL), RL)
            dst[rs, :] = src[rs].reshape(RL, H * D)
            return carry
        lax.fori_loop(0, nrows // RL, body, 0)

    @pl.when(h == 0)
    def _():
        copies[8].start()
        for cp in copies[:8]:
            cp.start()
        copies[0].wait()
        copies[1].wait()
        copies[8].wait()
        wg_s[0:3 * M, :] = wqkv_v[...].T
        wg_s[3 * M:MG, :] = jnp.broadcast_to(g_v[...], (16, M))
        kv_s[...] = jnp.zeros_like(kv_s)

        def b1(j, carry):
            cs = pl.ds(pl.multiple_of(j * CB, CB), CB)
            xt_c = xt_v[0, :, cs]
            t = _dot(wg_s[...], xt_c)
            pq_s[:, cs] = _phi(t[0:M]).astype(bf16)
            pk = _phi(t[M:2 * M]).astype(bf16)
            vt = jnp.concatenate([t[2 * M:3 * M].astype(bf16), jnp.ones((16, CB), bf16)], axis=0)
            kv_s[...] += _dot_nt(vt, pk)
            gate_s[:, cs] = jax.nn.sigmoid(t[3 * M:3 * M + 8])
            x_s[cs, :] = xt_c.T
            acc_s[:, cs] = jnp.zeros((M, CB), f32)
            return carry
        lax.fori_loop(0, NCB, b1, 0)

        copies[2].wait()
        r = lax.broadcasted_iota(jnp.int32, (M, M), 0) // DH
        cc = lax.broadcasted_iota(jnp.int32, (M, M), 1) // DH
        bm = r == cc
        kvm = jnp.where(bm, kv_s[0:M, :], 0.0).astype(bf16)
        w3_s[...] = lax.dot_general(wob_v[...], kvm, TN, preferred_element_type=f32).astype(bf16)
        zm_s[...] = jnp.where(bm, kv_s[M:M + 1, :], 0.0).astype(bf16)

        copies[3].wait()
        relayout(wk_s, wk_v, DC)

        def b2(j, carry):
            cs = pl.ds(pl.multiple_of(j * CB, CB), CB)
            pq = pq_s[:, cs]
            den = _dot(zm_s[...], pq) + 1e-6
            pqn = (pq.astype(f32) / den).astype(bf16)
            bt = _dot(w3_s[...], pqn)
            accb_s[:, cs] = (1.0 - gate_s[0:1, cs]) * bt
            return carry
        lax.fori_loop(0, NCB, b2, 0)

        copies[4].wait()
        relayout(wv_s, wv_v, DC)
        copies[5].wait()
        relayout(wq_s, wq_v, M)
        copies[6].wait()
        copies[7].wait()

    col = pl.ds(pl.multiple_of(h * D, D), D)
    q_s[...] = (_dot(x_s[...], wq_s[:, col]) * (D ** -0.5)).astype(bf16)
    k_s[...] = _dot(c_v[0], wk_s[:, col]).astype(bf16)
    v_s[...] = _dot(c_v[0], wv_s[:, col]).astype(bf16)

    row = lax.broadcasted_iota(jnp.int32, (T, T), 0)
    colid = lax.broadcasted_iota(jnp.int32, (T, T), 1)
    cmask = colid <= row

    for g in range(NTILE // 2):
        k0, r1 = 2 * g * T, (2 * g + 1) * T
        s_s[r1:S, k0:k0 + 2 * T] = _dot_nt(q_s[r1:S, :], k_s[k0:k0 + 2 * T, :])
        s_s[k0:r1, k0:r1] = _dot_nt(q_s[k0:r1, :], k_s[k0:r1, :])
    for t in range(NTILE):
        kl = t * T
        sd = jnp.where(cmask, s_s[kl:kl + T, kl:kl + T], -1e9)
        m = jnp.max(sd, axis=-1, keepdims=True)
        if kl > 0:
            so = s_s[kl:kl + T, 0:kl]
            m = jnp.maximum(m, jnp.max(so, axis=-1, keepdims=True))
        pd = jnp.exp(sd - m)
        l = jnp.sum(pd, axis=-1, keepdims=True)
        p_s[kl:kl + T, kl:kl + T] = pd.astype(bf16)
        if kl > 0:
            po = jnp.exp(so - m)
            l = l + jnp.sum(po, axis=-1, keepdims=True)
            p_s[kl:kl + T, 0:kl] = po.astype(bf16)
        l_s[kl:kl + T, :] = l
    pieces = [None] * NTILE

    def addp(u, blk):
        pieces[u] = blk if pieces[u] is None else pieces[u] + blk
    for g in range(NTILE // 2):
        k0, r1 = 2 * g * T, (2 * g + 1) * T
        c2 = _dot(p_s[r1:S, k0:k0 + 2 * T], v_s[k0:k0 + 2 * T, :])
        for u in range(2 * g + 1, NTILE):
            addp(u, c2[(u - 2 * g - 1) * T:(u - 2 * g) * T])
        addp(2 * g, _dot(p_s[k0:r1, k0:r1], v_s[k0:r1, :]))
    for t in range(NTILE):
        ctx_s[t * T:(t + 1) * T, :] = (pieces[t] / l_s[t * T:(t + 1) * T, :]).astype(bf16)

    acc_s[...] += _dot_nt(wot_v[h], ctx_s[...])

    @pl.when(h == H - 1)
    def _():
        outs = []
        for j in range(NCB):
            cs = pl.ds(j * CB, CB)
            o_s[:, cs] = (gate_s[0:1, cs] * acc_s[:, cs] + accb_s[:, cs]).astype(bf16)
            cp = pltpu.make_async_copy(o_s.at[:, cs], o_hbm.at[0, :, cs], osems.at[j])
            cp.start()
            outs.append(cp)
        for cp in outs:
            cp.wait()


@jax.jit
def pallas_gated_mix__compressed_kv_cla__linear_attn_block__prompt_kernel(A_x, A_c_kv, A_w_q, A_w_uk, A_w_uv, A_w_o, B_x, B_wqkv, B_wo, gate_w):
    args = (jnp.swapaxes(A_x, 1, 2), A_c_kv, A_w_q, A_w_uk, A_w_uv, jnp.swapaxes(A_w_o, 1, 2),
            B_wqkv, B_wo, gate_w.reshape(1, M))
    out_t = pl.pallas_call(
        kernel,
        grid=(H,),
        in_specs=[pl.BlockSpec(memory_space=pl.ANY) for _ in args],
        out_specs=pl.BlockSpec(memory_space=pl.ANY),
        out_shape=jax.ShapeDtypeStruct((1, M, S), bf16),
        scratch_shapes=[pltpu.VMEM(a.shape, a.dtype) for a in args] + [
            pltpu.SemaphoreType.DMA((9,)),
            pltpu.SemaphoreType.DMA((NCB,)),
            pltpu.VMEM((S, M), bf16),
            pltpu.VMEM((M, H * D), bf16),
            pltpu.VMEM((DC, H * D), bf16),
            pltpu.VMEM((DC, H * D), bf16),
            pltpu.VMEM((S, D), bf16),
            pltpu.VMEM((S, D), bf16),
            pltpu.VMEM((S, D), bf16),
            pltpu.VMEM((S, D), bf16),
            pltpu.VMEM((M, S), f32),
            pltpu.VMEM((MG, M), bf16),
            pltpu.VMEM((M, S), bf16),
            pltpu.VMEM((MV, M), f32),
            pltpu.VMEM((M, M), bf16),
            pltpu.VMEM((M, M), bf16),
            pltpu.VMEM((8, S), f32),
            pltpu.VMEM((M, S), f32),
            pltpu.VMEM((S, S), f32),
            pltpu.VMEM((S, S), bf16),
            pltpu.VMEM((S, 1), f32),
            pltpu.VMEM((M, S), bf16),
        ],
        compiler_params=pltpu.CompilerParams(
            dimension_semantics=("arbitrary",),
            vmem_limit_bytes=120 * 1024 * 1024,
        ),
    )(*args)
    return jnp.swapaxes(out_t, 1, 2)
```

```python
import jax
import jax.numpy as jnp
from jax import lax
import jax.experimental.pallas as pl
import jax.experimental.pallas.tpu as pltpu

S = 2048
M = 448
H = 16
D = 256
DC = 1024
DH = 28
T = 128
NTILE = S // T
CB = 512
NCB = S // CB
MG = 3 * M + 16
MV = M + 16
RL = 64

f32 = jnp.float32
bf16 = jnp.bfloat16
NT = (((1,), (1,)), ((), ()))
TN = (((0,), (0,)), ((), ()))


def _dot(a, b):
    return jnp.dot(a, b, preferred_element_type=f32)


def _dot_nt(a, b):
    return lax.dot_general(a, b, NT, preferred_element_type=f32)


def _phi(t):
    return jnp.where(t > 0, t + 1.0, jnp.exp(t)) + 1e-6


def kernel(xt_hbm, c_hbm, wq_hbm, wk_hbm, wv_hbm, wot_hbm, wqkv_hbm, wob_hbm, g_hbm, o_hbm,
           xt_v, c_v, wq_v, wk_v, wv_v, wot_v, wqkv_v, wob_v, g_v, sems, osems,
           x_s, wq_s, wk_s, wv_s, q_s, k_s, v_s, ctx_s, acc_s,
           wg_s, pq_s, kv_s, w3_s, zm_s, e_s, gate_s, accb_s, s_s, p_s, l_s, o_s):
    h = pl.program_id(0)

    srcs = (wqkv_hbm, g_hbm, wob_hbm, wk_hbm, wv_hbm, wq_hbm, c_hbm, wot_hbm, xt_hbm)
    dsts = (wqkv_v, g_v, wob_v, wk_v, wv_v, wq_v, c_v, wot_v, xt_v)
    copies = [pltpu.make_async_copy(s, d, sems.at[i]) for i, (s, d) in enumerate(zip(srcs, dsts))]

    def relayout(dst, src, nrows):
        def body(j, carry):
            rs = pl.ds(pl.multiple_of(j * RL, RL), RL)
            dst[rs, :] = src[rs].reshape(RL, H * D)
            return carry
        lax.fori_loop(0, nrows // RL, body, 0)

    @pl.when(h == 0)
    def _():
        copies[0].start()
        copies[1].start()
        copies[8].start()
        for cp in copies[2:8]:
            cp.start()
        copies[0].wait()
        copies[1].wait()
        wg_s[0:3 * M, :] = wqkv_v[...].T
        wg_s[3 * M:MG, :] = jnp.broadcast_to(g_v[...], (16, M))
        kv_s[...] = jnp.zeros_like(kv_s)
        copies[8].wait()

        def b1(j, carry):
            cs = pl.ds(pl.multiple_of(j * CB, CB), CB)
            xt_c = xt_v[0, :, cs]
            t = _dot(wg_s[...], xt_c)
            pq_s[:, cs] = _phi(t[0:M]).astype(bf16)
            pk = _phi(t[M:2 * M]).astype(bf16)
            vt = jnp.concatenate([t[2 * M:3 * M].astype(bf16), jnp.ones((16, CB), bf16)], axis=0)
            kv_s[...] += _dot_nt(vt, pk)
            gate_s[:, cs] = jax.nn.sigmoid(t[3 * M:3 * M + 8])
            x_s[cs, :] = xt_c.T
            acc_s[:, cs] = jnp.zeros((M, CB), f32)
            return carry
        lax.fori_loop(0, NCB, b1, 0)

        copies[2].wait()
        r = lax.broadcasted_iota(jnp.int32, (M, M), 0) // DH
        cc = lax.broadcasted_iota(jnp.int32, (M, M), 1) // DH
        bm = r == cc
        kvm = jnp.where(bm, kv_s[0:M, :], 0.0).astype(bf16)
        w3_s[...] = lax.dot_general(wob_v[...], kvm, TN, preferred_element_type=f32).astype(bf16)
        hz = lax.broadcasted_iota(jnp.int32, (H, M), 0) == lax.broadcasted_iota(jnp.int32, (H, M), 1) // DH
        zm_s[...] = jnp.where(hz, kv_s[M:M + 1, :], 0.0).astype(bf16)
        he = lax.broadcasted_iota(jnp.int32, (M, 2 * H), 0) // DH == lax.broadcasted_iota(jnp.int32, (M, 2 * H), 1) % H
        e_s[...] = jnp.where(he, 1.0, 0.0).astype(bf16)

        copies[3].wait()
        relayout(wk_s, wk_v, DC)

        def b2(j, carry):
            cs = pl.ds(pl.multiple_of(j * CB, CB), CB)
            pq = pq_s[:, cs]
            rc = 1.0 / (_dot(zm_s[...], pq) + 1e-6)
            rhi = rc.astype(bf16)
            rlo = (rc - rhi.astype(f32)).astype(bf16)
            rexp = _dot(e_s[...], jnp.concatenate([rhi, rlo], axis=0))
            pqn = (pq.astype(f32) * rexp).astype(bf16)
            bt = _dot(w3_s[...], pqn)
            accb_s[:, cs] = (1.0 - gate_s[0:1, cs]) * bt
            return carry
        lax.fori_loop(0, NCB, b2, 0)

        copies[4].wait()
        relayout(wv_s, wv_v, DC)
        copies[5].wait()
        relayout(wq_s, wq_v, M)
        copies[6].wait()
        copies[7].wait()

    col = pl.ds(pl.multiple_of(h * D, D), D)
    q_s[...] = (_dot(x_s[...], wq_s[:, col]) * (D ** -0.5)).astype(bf16)
    k_s[...] = _dot(c_v[0], wk_s[:, col]).astype(bf16)
    v_s[...] = _dot(c_v[0], wv_s[:, col]).astype(bf16)

    row = lax.broadcasted_iota(jnp.int32, (T, T), 0)
    colid = lax.broadcasted_iota(jnp.int32, (T, T), 1)
    cmask = colid <= row

    for g in range(NTILE // 2):
        k0, r1 = 2 * g * T, (2 * g + 1) * T
        s_s[r1:S, k0:k0 + 2 * T] = _dot_nt(q_s[r1:S, :], k_s[k0:k0 + 2 * T, :])
        s_s[k0:r1, k0:r1] = _dot_nt(q_s[k0:r1, :], k_s[k0:r1, :])
    for t in range(NTILE):
        kl = t * T
        sd = jnp.where(cmask, s_s[kl:kl + T, kl:kl + T], -1e9)
        m = jnp.max(sd, axis=-1, keepdims=True)
        if kl > 0:
            so = s_s[kl:kl + T, 0:kl]
            m = jnp.maximum(m, jnp.max(so, axis=-1, keepdims=True))
        pd = jnp.exp(sd - m)
        l = jnp.sum(pd, axis=-1, keepdims=True)
        p_s[kl:kl + T, kl:kl + T] = pd.astype(bf16)
        if kl > 0:
            po = jnp.exp(so - m)
            l = l + jnp.sum(po, axis=-1, keepdims=True)
            p_s[kl:kl + T, 0:kl] = po.astype(bf16)
        l_s[kl:kl + T, :] = l
    pieces = [None] * NTILE

    def addp(u, blk):
        pieces[u] = blk if pieces[u] is None else pieces[u] + blk
    for g in range(NTILE // 2):
        k0, r1 = 2 * g * T, (2 * g + 1) * T
        c2 = _dot(p_s[r1:S, k0:k0 + 2 * T], v_s[k0:k0 + 2 * T, :])
        for u in range(2 * g + 1, NTILE):
            addp(u, c2[(u - 2 * g - 1) * T:(u - 2 * g) * T])
        addp(2 * g, _dot(p_s[k0:r1, k0:r1], v_s[k0:r1, :]))
    for t in range(NTILE):
        ctx_s[t * T:(t + 1) * T, :] = (pieces[t] / l_s[t * T:(t + 1) * T, :]).astype(bf16)

    acc_s[...] += _dot_nt(wot_v[h], ctx_s[...])

    @pl.when(h == H - 1)
    def _():
        outs = []
        for j in range(NCB):
            cs = pl.ds(j * CB, CB)
            o_s[:, cs] = (gate_s[0:1, cs] * acc_s[:, cs] + accb_s[:, cs]).astype(bf16)
            cp = pltpu.make_async_copy(o_s.at[:, cs], o_hbm.at[0, :, cs], osems.at[j])
            cp.start()
            outs.append(cp)
        for cp in outs:
            cp.wait()


@jax.jit
def pallas_gated_mix__compressed_kv_cla__linear_attn_block__prompt_kernel(A_x, A_c_kv, A_w_q, A_w_uk, A_w_uv, A_w_o, B_x, B_wqkv, B_wo, gate_w):
    args = (jnp.swapaxes(A_x, 1, 2), A_c_kv, A_w_q, A_w_uk, A_w_uv, jnp.swapaxes(A_w_o, 1, 2),
            B_wqkv, B_wo, gate_w.reshape(1, M))
    out_t = pl.pallas_call(
        kernel,
        grid=(H,),
        in_specs=[pl.BlockSpec(memory_space=pl.ANY) for _ in args],
        out_specs=pl.BlockSpec(memory_space=pl.ANY),
        out_shape=jax.ShapeDtypeStruct((1, M, S), bf16),
        scratch_shapes=[pltpu.VMEM(a.shape, a.dtype) for a in args] + [
            pltpu.SemaphoreType.DMA((9,)),
            pltpu.SemaphoreType.DMA((NCB,)),
            pltpu.VMEM((S, M), bf16),
            pltpu.VMEM((M, H * D), bf16),
            pltpu.VMEM((DC, H * D), bf16),
            pltpu.VMEM((DC, H * D), bf16),
            pltpu.VMEM((S, D), bf16),
            pltpu.VMEM((S, D), bf16),
            pltpu.VMEM((S, D), bf16),
            pltpu.VMEM((S, D), bf16),
            pltpu.VMEM((M, S), f32),
            pltpu.VMEM((MG, M), bf16),
            pltpu.VMEM((M, S), bf16),
            pltpu.VMEM((MV, M), f32),
            pltpu.VMEM((M, M), bf16),
            pltpu.VMEM((H, M), bf16),
            pltpu.VMEM((M, 2 * H), bf16),
            pltpu.VMEM((8, S), f32),
            pltpu.VMEM((M, S), f32),
            pltpu.VMEM((S, S), f32),
            pltpu.VMEM((S, S), bf16),
            pltpu.VMEM((S, 1), f32),
            pltpu.VMEM((M, S), bf16),
        ],
        compiler_params=pltpu.CompilerParams(
            dimension_semantics=("arbitrary",),
            vmem_limit_bytes=120 * 1024 * 1024,
        ),
    )(*args)
    return jnp.swapaxes(out_t, 1, 2)
```
